```python
import os as _os
_os.environ.setdefault("JAX_PLATFORMS", "cpu")
import jax
import jax.numpy as jnp

def _softmax(x, axis=-1):
    return jax.nn.softmax(x, axis=axis)
def _gelu(x):
    return jax.nn.gelu(x, approximate=True)
def _silu(x):
    return jax.nn.silu(x)
def _sigmoid(x):
    return jax.nn.sigmoid(x)
def _layernorm(x, axis=-1, eps=1e-5):
    m = jnp.mean(x, axis=axis, keepdims=True)
    v = jnp.var(x, axis=axis, keepdims=True)
    return (x - m) / jnp.sqrt(v + eps)
def _scatter_add(tgt, idx, src, axis=0):
    return tgt.at[idx].add(src)
def _segment_sum(src, seg, n):
    return jax.ops.segment_sum(src, seg, n)
class _Rng:
    def __init__(self, key):
        self._k = key
    def _next(self):
        self._k, sub = jax.random.split(self._k)
        return sub
    def normal(self, shape):
        return jax.random.normal(self._next(), shape, dtype=jnp.bfloat16)
    def randint(self, lo, hi, shape):
        return jax.random.randint(self._next(), shape, lo, hi, dtype=jnp.int32)
    def uniform(self, shape, lo=0.0, hi=1.0):
        return jax.random.uniform(self._next(), shape, jnp.bfloat16, lo, hi)
    def permutation(self, n):
        return jax.random.permutation(self._next(), n)


kernel_name = 'sequential_preLN__linear_attn_block__glu_gated_reglu__prompt'

def setup_inputs():
    _rng = _Rng(jax.random.key(int.from_bytes(__import__("os").urandom(4), "little")))
    _w = (lambda a: (lambda t: t.astype(jnp.bfloat16) if jnp.issubdtype(t.dtype, jnp.floating) else t)(jnp.asarray(a)))
    def _A_setup():
        B, S, D = 1, 2048, 640
        return {
            "x": _w((lambda *s: _rng.normal(s) * 0.05)(B, S, D)),
            "wqkv": _w((lambda *s: _rng.normal(s) * 0.05)(D, 3 * D)),
            "wo": _w((lambda *s: _rng.normal(s) * 0.05)(D, D)),
        }
    _A_in = _A_setup()

    def _B_setup():
        B, S, D, F = 1, 2048, 640, 1536
        return {
            "x": _w((lambda *s: _rng.normal(s) * 0.05)(B, S, D)),
            "W_gate": _w((lambda *s: _rng.normal(s) * 0.05)(D, F) * (2.0 / D) ** 0.5),
            "W_up": _w((lambda *s: _rng.normal(s) * 0.05)(D, F) * (2.0 / D) ** 0.5),
            "W_down": _w((lambda *s: _rng.normal(s) * 0.05)(F, D) * (1.0 / F) ** 0.5),
        }
    _B_in = _B_setup()

    return {
        "A_x": _A_in["x"],
        "A_wqkv": _A_in["wqkv"],
        "A_wo": _A_in["wo"],
        "B_x": _B_in["x"],
        "B_W_gate": _B_in["W_gate"],
        "B_W_up": _B_in["W_up"],
        "B_W_down": _B_in["W_down"],
    }

def reference(A_x, A_wqkv, A_wo, B_x, B_W_gate, B_W_up, B_W_down):
    def _A_ref(x, wqkv, wo):
        B, S, D = x.shape
        H = 32; Dh = D // H
        qkv = (lambda x, *d: x.transpose(*d))((x @ wqkv).reshape(B, S, 3, H, Dh), 2, 0, 3, 1, 4)
        q, k, v = qkv[0], qkv[1], qkv[2]
        phi = lambda t: jnp.where(t > 0, t + 1, jnp.exp(t)) + 1e-6
        pq, pk = phi(q), phi(k)
        kv = jnp.einsum("bhsd,bhse->bhde", pk, v)
        z = jnp.einsum("bhsd->bhd", pk)
        num = jnp.einsum("bhqd,bhde->bhqe", pq, kv)
        den = jnp.einsum("bhqd,bhd->bhq", pq, z)[..., None] + 1e-6
        o = num / den
        return (lambda x, *d: x.transpose(*d))(o, 0, 2, 1, 3).reshape(B, S, D) @ wo

    def _B_ref(x, W_gate, W_up, W_down):
        gate = jnp.einsum("bsd,df->bsf", x, W_gate)
        up = jnp.einsum("bsd,df->bsf", x, W_up)
        gate = gate * (lambda x, dt: x.astype(dt))(gate > 0, gate.dtype)
        h = gate * up
        return jnp.einsum("bsf,fd->bsd", h, W_down)

    x = A_x
    h = x + _A_ref(_layernorm(x, axis=-1), A_wqkv, A_wo)
    h2 = h + _B_ref(_layernorm(h, axis=-1), B_W_gate, B_W_up, B_W_down)
    return h2
```

```python
import jax
import jax.numpy as jnp
from jax import lax
import jax.experimental.pallas as pl
import jax.experimental.pallas.tpu as pltpu

S, D, H, DH, F = 2048, 640, 32, 20, 1536
TM = 512
NT = S // TM
FC = 512
NC = F // FC
NL = D // 128
RANGES = [(0, 144), (112, 272), (240, 400), (368, 528), (496, 640)]
TAIL = [(0, 256), (256, 384), (384, 512)]
LN2 = [('dn', 0)]
ATTN_C = 0

NT_DIMS = (((1,), (1,)), ((), ()))
f32, bf16 = jnp.float32, jnp.bfloat16
PET = dict(preferred_element_type=f32)


def _ln(x):
    mu = jnp.mean(x, axis=-1, keepdims=True)
    xc = x - mu
    var = jnp.mean(xc * xc, axis=-1, keepdims=True)
    return xc * lax.rsqrt(var + 1e-5)


def _phi(t):
    return jnp.where(t > 0, t + 1.0, jnp.exp(t)) + 1e-6


def _permute_rows(src_ref, dst_ref):
    for t in range(NL):
        for d in range(DH):
            parts = [src_ref[t, pl.ds(hb * 8 * DH + d, 8, stride=DH), :] for hb in range(H // 8)]
            dst_ref[d * H:(d + 1) * H, t * 128:(t + 1) * 128] = jnp.concatenate(parts, axis=0).astype(bf16)


def kern(x_hbm, wqkv_hbm, wo_hbm, wg_hbm, wu_hbm, wd_hbm, out_hbm,
         x_v, wq_v, wk_v, wv_v, wo_v, wg_v, wu_v, wd_v, xn_v, wkT_v, wqTp_v, tmp_v, m_v, pq_v, h_v, hn_v, o_v,
         sems, osems):
    xcp = [pltpu.make_async_copy(x_hbm.at[pl.ds(i * TM, TM)], x_v.at[pl.ds(i * TM, TM)], sems.at[i]) for i in range(NT)]
    wqc, wkc, wvc = [pltpu.make_async_copy(wqkv_hbm.at[:, pl.ds(j * D, D)], r, sems.at[NT + j])
                     for j, r in enumerate([wq_v, wk_v, wv_v])]
    woc, wgc, wuc, wdc = [pltpu.make_async_copy(a, b, sems.at[NT + 3 + j]) for j, (a, b) in enumerate(
        [(wo_hbm, wo_v), (wg_hbm, wg_v), (wu_hbm, wu_v), (wd_hbm, wd_v)])]

    def rows(i):
        if isinstance(i, int):
            return pl.ds(i * TM, TM)
        return pl.ds(pl.multiple_of(i * TM, TM), TM)

    def ln_rows(a, n=TM // 2):
        r = pl.ds(a, n)
        xn = _ln(x_v[r, :].astype(f32)).astype(bf16)
        xn_v[r, :] = xn
        return xn

    def vmm(xn):
        return jnp.dot(xn, wv_v[...], **PET).astype(bf16)

    def cat(*p, axis=0):
        return jnp.concatenate(p, axis=axis)

    kv = [None] * NL
    z = None

    def k_tile(xn):
        nonlocal z
        pkT = _phi(lax.dot_general(wkT_v[...], xn, NT_DIMS, **PET))
        zi = pkT[:, 0:128]
        for c in range(1, xn.shape[0] // 128):
            zi = zi + pkT[:, c * 128:(c + 1) * 128]
        z = zi if z is None else z + zi
        return pkT.astype(bf16)

    def kv_tile(pkTb, v):
        for j, (a, b) in enumerate(RANGES):
            p = jnp.dot(pkTb[a:b], v[:, j * 128:(j + 1) * 128], **PET)
            kv[j] = p if kv[j] is None else kv[j] + p

    def q_tile(i):
        pq_v[rows(i), :] = _phi(lax.dot_general(xn_v[rows(i), :], wqTp_v[...], NT_DIMS, **PET))

    xcp[0].start()
    wvc.start()
    xcp[0].wait()
    wkc.start()
    xn0 = ln_rows(0, TM)
    wvc.wait()
    va = jnp.dot(xn0, wv_v[:, :512], **PET).astype(bf16)
    wkc.wait()
    xcp[1].start(); xcp[2].start()
    vb = jnp.dot(xn0, wv_v[:, 512:], **PET).astype(bf16)
    wkT_v[...] = wk_v[...].astype(f32).T.astype(bf16)
    v0 = cat(va, vb, axis=1)
    pk0a = k_tile(xn0[:384])
    xcp[1].wait()
    xcp[3].start(); wqc.start()
    pk0b = k_tile(xn0[384:])
    xn1a = ln_rows(512)
    v1a = vmm(xn1a)
    xn1b = ln_rows(768)
    v1b = vmm(xn1b)
    xn1 = cat(xn1a, xn1b); v1 = cat(v1a, v1b)
    xcp[2].wait(); xcp[3].wait(); wqc.wait()
    woc.start(); wgc.start(); wuc.start(); wdc.start()
    kv_tile(cat(pk0a, pk0b, axis=1), v0)
    pk1 = k_tile(xn1)
    xn2 = ln_rows(1024, TM)
    v2 = vmm(xn2)
    xn3 = ln_rows(1536, TM)
    kv_tile(pk1, v1)
    pk2 = k_tile(xn2)
    v3 = vmm(xn3)
    wqT = wq_v[...].astype(f32).T
    for t in range(NL):
        tmp_v[t] = wqT[:, t * 128:(t + 1) * 128]
    _permute_rows(tmp_v, wqTp_v)
    woc.wait(); wgc.wait(); wuc.wait(); wdc.wait()
    kv_tile(pk2, v2)
    pk3 = k_tile(xn3)
    q_tile(0)
    kv_tile(pk3, v3)
    zc = jnp.broadcast_to(jnp.sum(z, axis=1, keepdims=True), (D, 128))
    tmp_v[0] = zc
    zp = jnp.concatenate([tmp_v[0, pl.ds(hb * 8 * DH + d, 8, stride=DH), :]
                          for d in range(DH) for hb in range(H // 8)], axis=0)
    zrow = zp.T[0:1, :]
    q_tile(1)
    for t in range(NL):
        tmp_v[t] = jnp.zeros((D, 128), f32)
    for j, (a, b) in enumerate(RANGES):
        d_id = (lax.broadcasted_iota(jnp.int32, (b - a, 128), 0) + a) // DH
        e_id = (lax.broadcasted_iota(jnp.int32, (b - a, 128), 1) + j * 128) // DH
        kvm = jnp.where(d_id == e_id, kv[j], 0.0).astype(bf16)
        mp = jnp.dot(kvm, wo_v[j * 128:(j + 1) * 128, :], **PET)
        for t in range(NL):
            tmp_v[t, a:b, :] += mp[:, t * 128:(t + 1) * 128]
    _permute_rows(tmp_v, m_v)

    def pqn_tile(i):
        pq = pq_v[rows(i), :]
        p = pq * zrow
        s = p[:, 0:128]
        for t in range(1, NL):
            s = s + p[:, t * 128:(t + 1) * 128]
        s = s + pltpu.roll(s, 64, 1)
        s = s + pltpu.roll(s, 32, 1)
        inv = 1.0 / (s + 1e-6)
        return jnp.concatenate([(pq[:, t * 128:(t + 1) * 128] * inv).astype(bf16) for t in range(NL)], axis=1)

    def attn_tile(i, pqn):
        h = x_v[rows(i), :].astype(f32) + jnp.dot(pqn, m_v[...], **PET)
        return h

    pqn = pqn_tile(0)
    q_tile(2)
    h = attn_tile(0, pqn)
    h_v[...] = h
    q_tile(3)
    hn_v[...] = _ln(h).astype(bf16)

    ocp = []

    def mlp_tile(i, last):
        acc = h_v[...]
        hn = hn_v[...]
        h = None
        nch = TM // len(LN2)

        def ln2(stage, c):
            for n, (s, cc) in enumerate(LN2):
                if s == stage and cc == c:
                    hn_v[n * nch:(n + 1) * nch, :] = _ln(h[n * nch:(n + 1) * nch]).astype(bf16)

        for c in range(NC):
            g = jnp.dot(hn, wg_v[:, c * FC:(c + 1) * FC], **PET)
            if not last and h is not None:
                ln2('g', c)
            u = jnp.dot(hn, wu_v[:, c * FC:(c + 1) * FC], **PET)
            if not last and h is not None:
                ln2('u', c)
            if c == ATTN_C and not last:
                pqn = pqn_tile(i + 1)
            hid = (jnp.maximum(g, 0.0) * u).astype(bf16)
            if c == ATTN_C and not last:
                h = attn_tile(i + 1, pqn)
            if last and c == NC - 1:
                break
            acc = acc + jnp.dot(hid, wd_v[c * FC:(c + 1) * FC, :], **PET)
            if c == ATTN_C and not last:
                h_v[...] = h
            if not last and h is not None:
                ln2('dn', c)
        if not last:
            o_v[rows(i), :] = acc.astype(bf16)
            pltpu.make_async_copy(o_v.at[rows(i)], out_hbm.at[rows(i)], osems.at[i]).start()
        else:
            for n, (a, b) in enumerate(TAIL):
                r = pl.ds(i * TM + a, b - a)
                o_v[r, :] = (acc[a:b] + jnp.dot(hid[a:b], wd_v[(NC - 1) * FC:, :], **PET)).astype(bf16)
                cp = pltpu.make_async_copy(o_v.at[r], out_hbm.at[r], osems.at[i + n])
                cp.start()
                ocp.append(cp)

    for i in range(NT - 1):
        mlp_tile(i, False)
    mlp_tile(NT - 1, True)
    for i in range(NT - 1):
        pltpu.make_async_copy(o_v.at[rows(i)], out_hbm.at[rows(i)], osems.at[i]).wait()
    for cp in ocp:
        cp.wait()


@jax.jit
def pallas_sequential_preLN__linear_attn_block__glu_gated_reglu__prompt_kernel(
        A_x, A_wqkv, A_wo, B_x, B_W_gate, B_W_up, B_W_down):
    x = A_x.reshape(S, D)
    anyspec = pl.BlockSpec(memory_space=pl.ANY)
    out = pl.pallas_call(
        kern,
        out_shape=jax.ShapeDtypeStruct((S, D), bf16),
        in_specs=[anyspec] * 6,
        out_specs=anyspec,
        scratch_shapes=[
            pltpu.VMEM((S, D), bf16), pltpu.VMEM((D, D), bf16), pltpu.VMEM((D, D), bf16), pltpu.VMEM((D, D), bf16),
            pltpu.VMEM((D, D), bf16),
            pltpu.VMEM((D, F), bf16), pltpu.VMEM((D, F), bf16), pltpu.VMEM((F, D), bf16),
            pltpu.VMEM((S, D), bf16), pltpu.VMEM((D, D), bf16), pltpu.VMEM((D, D), bf16),
            pltpu.VMEM((NL, D, 128), f32),
            pltpu.VMEM((D, D), bf16), pltpu.VMEM((S, D), f32), pltpu.VMEM((TM, D), f32), pltpu.VMEM((TM, D), bf16),
            pltpu.VMEM((S, D), bf16),
            pltpu.SemaphoreType.DMA((NT + 7,)), pltpu.SemaphoreType.DMA((NT + len(TAIL) - 1,)),
        ],
        compiler_params=pltpu.CompilerParams(vmem_limit_bytes=100 * 1024 * 1024, flags={'XLA_TPU_EVENLY_DISTRIBUTE_CRITICAL_NODES': True}),
    )(x, A_wqkv, A_wo, B_W_gate, B_W_up, B_W_down)
    return out.reshape(1, S, D)
```
